```python
import os as _os
_os.environ.setdefault("JAX_PLATFORMS", "cpu")
import jax
import jax.numpy as jnp

def _softmax(x, axis=-1):
    return jax.nn.softmax(x, axis=axis)
def _gelu(x):
    return jax.nn.gelu(x, approximate=True)
def _silu(x):
    return jax.nn.silu(x)
def _sigmoid(x):
    return jax.nn.sigmoid(x)
def _layernorm(x, axis=-1, eps=1e-5):
    m = jnp.mean(x, axis=axis, keepdims=True)
    v = jnp.var(x, axis=axis, keepdims=True)
    return (x - m) / jnp.sqrt(v + eps)
def _scatter_add(tgt, idx, src, axis=0):
    return tgt.at[idx].add(src)
def _segment_sum(src, seg, n):
    return jax.ops.segment_sum(src, seg, n)
class _Rng:
    def __init__(self, key):
        self._k = key
    def _next(self):
        self._k, sub = jax.random.split(self._k)
        return sub
    def normal(self, shape):
        return jax.random.normal(self._next(), shape, dtype=jnp.bfloat16)
    def randint(self, lo, hi, shape):
        return jax.random.randint(self._next(), shape, lo, hi, dtype=jnp.int32)
    def uniform(self, shape, lo=0.0, hi=1.0):
        return jax.random.uniform(self._next(), shape, jnp.bfloat16, lo, hi)
    def permutation(self, n):
        return jax.random.permutation(self._next(), n)


kernel_name = 'concat_heads__spectral_gfnet__sliding_block__prompt'

def setup_inputs():
    _rng = _Rng(jax.random.key(int.from_bytes(__import__("os").urandom(4), "little")))
    _w = (lambda a: (lambda t: t.astype(jnp.bfloat16) if jnp.issubdtype(t.dtype, jnp.floating) else t)(jnp.asarray(a)))
    def _A_setup():
        B, S, D = 1, 2048, 640
        Df = D // 2 + 1
        return {
            "x": _w((lambda *s: _rng.normal(s) * 0.05)(B, S, D)),
            "w_r": _w((lambda *s: _rng.normal(s) * 0.4)(S, Df) * 0.02),
            "w_i": _w((lambda *s: _rng.normal(s) * 0.4)(S, Df) * 0.02),
        }
    _A_in = _A_setup()

    def _B_setup():
        B, S, D = 1, 2048, 640
        return {
            "x": _w((lambda *s: _rng.normal(s) * 0.2)(B, S, D)),
            "wqkv": _w((lambda *s: _rng.normal(s) * 0.2)(D, 3 * D)),
            "wo": _w((lambda *s: _rng.normal(s) * 0.05)(D, D)),
        }
    _B_in = _B_setup()

    return {
        "A_x": _A_in["x"],
        "A_w_r": _A_in["w_r"],
        "A_w_i": _A_in["w_i"],
        "B_x": _B_in["x"],
        "B_wqkv": _B_in["wqkv"],
        "B_wo": _B_in["wo"],
    }

def reference(A_x, A_w_r, A_w_i, B_x, B_wqkv, B_wo):
    def _A_ref(x, w_r, w_i):
        B, S, D = x.shape
        X = (lambda x, axes=(-2,-1): jnp.fft.rfft2(x.astype(jnp.float32), axes=axes))(x, axes=(-2, -1))
        W = w_r + 1j * w_i
        X = X * W
        y = (lambda x, s, axes=(-2,-1): jnp.fft.irfft2(x, s=s, axes=axes).astype(jnp.bfloat16))(X, (S, D), axes=(-2, -1))
        return y

    def _B_ref(x, wqkv, wo):
        B, S, D = x.shape
        H = 32; Dh = D // H; W = 256
        qkv = (lambda x, *d: x.transpose(*d))((x @ wqkv).reshape(B, S, 3, H, Dh), 2, 0, 3, 1, 4)
        q, k, v = qkv[0], qkv[1], qkv[2]
        scores = jnp.einsum("bhqd,bhkd->bhqk", q, k) * (Dh ** -0.5)
        idx = jnp.arange(S)
        mask = (idx[:, None] - idx[None, :] >= 0) & (idx[:, None] - idx[None, :] < W)
        scores = jnp.where(mask[None, None], scores, -1e9)
        p = _softmax(scores, axis=-1)
        o = jnp.einsum("bhqk,bhkd->bhqd", p, v)
        return (lambda x, *d: x.transpose(*d))(o, 0, 2, 1, 3).reshape(B, S, D) @ wo

    a = _A_ref(A_x, A_w_r, A_w_i)
    b = _B_ref(B_x, B_wqkv, B_wo)
    return jnp.concatenate([a, b], axis=-1)
```

```python
import math

import numpy as np
import jax
import jax.numpy as jnp
from jax import lax
import jax.experimental.pallas as pl
import jax.experimental.pallas.tpu as pltpu

S = 2048
D = 640
DF = 321
LP = 384
H = 32
DH = 20
WIN = 256
BQ = 128
NB = 16
F32 = jnp.float32
BF16 = jnp.bfloat16


def _tables():
    d = np.arange(D)[:, None].astype(np.float64)
    k = np.arange(DF)[None, :].astype(np.float64)
    ang = 2.0 * np.pi * d * k / D
    fd = np.zeros((D, 2 * LP), np.float64)
    fd[:, :DF] = np.cos(ang)
    fd[:, LP:LP + DF] = -np.sin(ang)

    c = np.full((DF,), 2.0)
    c[0] = 1.0
    c[DF - 1] = 1.0
    gd = np.zeros((2 * LP, D), np.float64)
    gd[:DF, :] = (c[:, None] * np.cos(ang.T)) / (S * D)
    gi = -(c[:, None] * np.sin(ang.T)) / (S * D)
    gi[0, :] = 0.0
    gi[DF - 1, :] = 0.0
    gd[LP:LP + DF, :] = gi

    b = np.arange(16)[:, None, None].astype(np.float64)
    k2 = np.arange(128)[None, :, None].astype(np.float64)
    a = np.arange(128)[None, None, :].astype(np.float64)
    th = 2.0 * np.pi * (16.0 * a + b) * k2 / S
    mf = np.concatenate([np.cos(th), -np.sin(th)], axis=1)
    tht = np.transpose(th, (0, 2, 1))
    mi = np.concatenate([np.cos(tht), np.sin(tht)], axis=1)
    to = lambda z: np.asarray(z, np.float32)
    return to(fd), to(gd), to(mf), to(mi)


def _cmul_const(xr, xi, k, n, sign):
    k = k % n
    if k == 0:
        return xr, xi
    if 4 * k == n:
        return (-xi, xr) if sign > 0 else (xi, -xr)
    if 2 * k == n:
        return -xr, -xi
    if 4 * k == 3 * n:
        return (xi, -xr) if sign > 0 else (-xi, xr)
    cr = math.cos(2.0 * math.pi * k / n)
    ci = sign * math.sin(2.0 * math.pi * k / n)
    if abs(abs(cr) - abs(ci)) < 1e-12:
        if (cr > 0) == (ci > 0):
            return cr * (xr - xi), cr * (xr + xi)
        return cr * (xr + xi), cr * (xi - xr)
    return cr * xr - ci * xi, cr * xi + ci * xr


def _fft_list(xs, sign):
    n = len(xs)
    if n == 1:
        return xs
    ev = _fft_list(xs[0::2], sign)
    od = _fft_list(xs[1::2], sign)
    out = [None] * n
    for k in range(n // 2):
        er, ei = ev[k]
        tr, ti = _cmul_const(od[k][0], od[k][1], k, n, sign)
        out[k] = (er + tr, ei + ti)
        out[k + n // 2] = (er - tr, ei - ti)
    return out


def _kernel(ax_h, wr_h, wi_h, bx_h, wqkv_h, wo_h, fd_h, gd_h, mf_h, mi_h,
            out_h,
            ax_v, wr_v, wi_v, bx_v, wqkv_v, wo_v, fd_v, gd_v, mf_v, mi_v,
            oa_v, ob_v, wrn, win,
            u_scr, b_scr, k_scr, qt_scr, vt_scr, ot_scr, wt_scr, s_scr,
            sems):
    RC = 512
    NC = S // RC

    def full_cp(src, dst, i):
        return pltpu.make_async_copy(src, dst, sems.at[i])

    def rows_cp(src, dst, r, i):
        return pltpu.make_async_copy(src.at[pl.ds(r, RC)], dst.at[pl.ds(r, RC)], sems.at[i])

    def out_cp(src, col, r, i):
        return pltpu.make_async_copy(src.at[pl.ds(r, RC)],
                                     out_h.at[pl.ds(r, RC), pl.ds(col, D)], sems.at[i])

    SEM_WQKV, SEM_BX, SEM_WO, SEM_FD, SEM_AX, SEM_WR, SEM_WI = 0, 1, 5, 6, 7, 11, 12
    SEM_MF, SEM_MI, SEM_GD, SEM_OB, SEM_OA = 13, 14, 15, 16, 20

    full_cp(wqkv_h, wqkv_v, SEM_WQKV).start()
    for i in range(NC):
        rows_cp(bx_h, bx_v, i * RC, SEM_BX + i).start()
    full_cp(wo_h, wo_v, SEM_WO).start()
    full_cp(fd_h, fd_v, SEM_FD).start()
    for i in range(NC):
        rows_cp(ax_h, ax_v, i * RC, SEM_AX + i).start()
    full_cp(wr_h, wr_v, SEM_WR).start()
    full_cp(wi_h, wi_v, SEM_WI).start()
    full_cp(mf_h, mf_v, SEM_MF).start()
    full_cp(mi_h, mi_v, SEM_MI).start()
    full_cp(gd_h, gd_v, SEM_GD).start()

    full_cp(wqkv_h, wqkv_v, SEM_WQKV).wait()
    wt_scr[0] = wqkv_v[:, 0:D].astype(F32).T.astype(BF16)
    wt_scr[1] = wqkv_v[:, 2 * D:3 * D].astype(F32).T.astype(BF16)
    scale = DH ** -0.5
    nt = (((1,), (1,)), ((), ()))

    def b_proj(i, c):
        r = pl.multiple_of(i * RC, RC)
        rows_cp(bx_h, bx_v, r, SEM_BX + i).wait()
        x = bx_v[pl.ds(r, RC), :]
        k_scr[pl.ds(r, RC), :] = jnp.dot(
            x, wqkv_v[:, D:2 * D], preferred_element_type=F32).astype(BF16)
        qt = lax.dot_general(wt_scr[0], x, nt, preferred_element_type=F32)
        qt_scr[:, pl.ds(r, RC)] = (qt * scale).astype(BF16)
        vt = lax.dot_general(wt_scr[1], x, nt, preferred_element_type=F32)
        vt_scr[:, pl.ds(r, RC)] = vt.astype(BF16)
        return c
    with jax.named_scope("b_proj"):
        lax.fori_loop(0, NC, b_proj, 0)

    jj = lax.broadcasted_iota(jnp.int32, (BQ, BQ), 0)
    ii = lax.broadcasted_iota(jnp.int32, (BQ, BQ), 1)
    tri = jj <= ii

    def qk_block(t, nkb, slot):
        ks = t - (nkb - 1) * BQ
        for h in range(H):
            lo = h * DH
            c0 = (lo // 128) * 128
            c1 = ((lo + DH + 127) // 128) * 128
            wd = c1 - c0
            rows = lax.broadcasted_iota(jnp.int32, (wd, BQ), 0) + c0
            qt = qt_scr[c0:c1, pl.ds(t, BQ)]
            qtm = jnp.where((rows >= lo) & (rows < lo + DH), qt, jnp.zeros_like(qt))
            kk = k_scr[pl.ds(ks, nkb * BQ), c0:c1]
            s_scr[slot, h, 0:nkb * BQ, :] = jnp.dot(kk, qtm, preferred_element_type=F32)

    def sm_block(t, nkb, slot):
        ks = t - (nkb - 1) * BQ
        for h in range(H):
            lo = h * DH
            s_last = s_scr[slot, h, (nkb - 1) * BQ:nkb * BQ, :]
            if nkb == 3:
                cmb = jnp.where(tri, s_last, s_scr[slot, h, 0:BQ, :])
            else:
                cmb = jnp.where(tri, s_last, -1e30)
            m = jnp.max(cmb, axis=0, keepdims=True)
            if nkb >= 2:
                s_mid = s_scr[slot, h, (nkb - 2) * BQ:(nkb - 1) * BQ, :]
                m = jnp.maximum(m, jnp.max(s_mid, axis=0, keepdims=True))
            pc = jnp.exp(cmb - m)
            l = jnp.sum(pc, axis=0, keepdims=True)
            p_last = jnp.where(tri, pc, 0.0).astype(BF16)
            vt = vt_scr[lo:lo + DH, pl.ds(ks, nkb * BQ)]
            o = jnp.dot(vt[:, (nkb - 1) * BQ:], p_last, preferred_element_type=F32)
            if nkb >= 2:
                pm = jnp.exp(s_mid - m)
                l = l + jnp.sum(pm, axis=0, keepdims=True)
                o = o + jnp.dot(vt[:, (nkb - 2) * BQ:(nkb - 1) * BQ], pm.astype(BF16),
                                preferred_element_type=F32)
            if nkb == 3:
                p_first = jnp.where(tri, 0.0, pc).astype(BF16)
                o = o + jnp.dot(vt[:, :BQ], p_first, preferred_element_type=F32)
            ot_scr[lo:lo + DH, pl.ds(t, BQ)] = o / l

    qk_block(0, 1, 0)
    qk_block(BQ, 2, 1)
    sm_block(0, 1, 0)
    qk_block(2 * BQ, 3, 0)
    sm_block(BQ, 2, 1)

    def attn_loop(j, c):
        t = pl.multiple_of((2 * j + 3) * BQ, BQ)
        qk_block(t, 3, 1)
        sm_block(t - BQ, 3, 0)
        qk_block(t + BQ, 3, 0)
        sm_block(t, 3, 1)
        return c
    with jax.named_scope("attn_loop"):
        lax.fori_loop(0, 6, attn_loop, 0)
    qk_block(15 * BQ, 3, 1)
    sm_block(14 * BQ, 3, 0)
    sm_block(15 * BQ, 3, 1)

    full_cp(wo_h, wo_v, SEM_WO).wait()

    def b_out(i, c):
        r = pl.multiple_of(i * RC, RC)
        o = ot_scr[:, pl.ds(r, RC)].T.astype(BF16)
        y = jnp.dot(o, wo_v[...], preferred_element_type=F32)
        ob_v[pl.ds(r, RC), :] = y.astype(BF16)
        out_cp(ob_v, D, r, SEM_OB + i).start()
        return c
    with jax.named_scope("b_out"):
        lax.fori_loop(0, NC, b_out, 0)

    full_cp(fd_h, fd_v, SEM_FD).wait()
    full_cp(wr_h, wr_v, SEM_WR).wait()
    full_cp(wi_h, wi_v, SEM_WI).wait()

    def a_row(i, c):
        r = pl.multiple_of(i * RC, RC)
        rows_cp(ax_h, ax_v, r, SEM_AX + i).wait()
        u = jnp.dot(ax_v[pl.ds(r, RC), :], fd_v[...], preferred_element_type=F32)
        for j in range(6):
            u_scr[j, pl.ds(r, RC), :] = u[:, j * 128:(j + 1) * 128]
        for src, dst in ((wr_v, wrn), (wi_v, win)):
            main = src[0:256, pl.ds(r, RC)].astype(F32)
            dst[pl.ds(r, RC), 0:256] = main.T
            tail = src[256:DF, pl.ds(r, RC)].astype(F32)
            tail = jnp.concatenate([tail, jnp.zeros((LP - DF, RC), F32)], axis=0)
            dst[pl.ds(r, RC), 256:LP] = tail.T
        return c
    with jax.named_scope("a_row"):
        lax.fori_loop(0, NC, a_row, 0)

    full_cp(mf_h, mf_v, SEM_MF).wait()

    def a_colf(b, c):
        ub = jnp.concatenate([u_scr[j, pl.ds(b, 128, stride=16), :] for j in range(6)],
                             axis=1).astype(BF16)
        pq = jnp.dot(mf_v[b], ub, preferred_element_type=F32)
        p = pq[:128]
        q = pq[128:]
        b_scr[b, :, :LP] = p[:, :LP] - q[:, LP:]
        b_scr[b, :, LP:] = p[:, LP:] + q[:, :LP]
        return c
    with jax.named_scope("a_colf"):
        lax.fori_loop(0, 16, a_colf, 0)

    def a_mid(t, c):
        r = pl.multiple_of(t * 8, 8)
        for lc in range(3):
            lo = lc * 128
            xs = [(b_scr[b, pl.ds(r, 8), lo:lo + 128],
                   b_scr[b, pl.ds(r, 8), LP + lo:LP + lo + 128]) for b in range(16)]
            X = _fft_list(xs, -1)
            Y = []
            for k1 in range(16):
                wr = wrn[pl.ds(128 * k1 + r, 8), lo:lo + 128]
                wi = win[pl.ds(128 * k1 + r, 8), lo:lo + 128]
                xr, xi = X[k1]
                Y.append((xr * wr - xi * wi, xr * wi + xi * wr))
            C = _fft_list(Y, +1)
            for b in range(16):
                b_scr[b, pl.ds(r, 8), lo:lo + 128] = C[b][0]
                b_scr[b, pl.ds(r, 8), LP + lo:LP + lo + 128] = C[b][1]
        return c
    with jax.named_scope("a_mid"):
        lax.fori_loop(0, 16, a_mid, 0)

    full_cp(mi_h, mi_v, SEM_MI).wait()

    def a_coli(b, c):
        cb = b_scr[b].astype(BF16)
        pq = jnp.dot(mi_v[b], cb, preferred_element_type=F32)
        p = pq[:128]
        q = pq[128:]
        zr = p[:, :LP] - q[:, LP:]
        zi = p[:, LP:] + q[:, :LP]
        for j in range(3):
            u_scr[j, pl.ds(b, 128, stride=16), :] = zr[:, j * 128:(j + 1) * 128]
            u_scr[3 + j, pl.ds(b, 128, stride=16), :] = zi[:, j * 128:(j + 1) * 128]
        return c
    with jax.named_scope("a_coli"):
        lax.fori_loop(0, 16, a_coli, 0)

    full_cp(gd_h, gd_v, SEM_GD).wait()

    def a_rowi(i, c):
        r = pl.multiple_of(i * RC, RC)
        z = jnp.concatenate([u_scr[j, pl.ds(r, RC), :] for j in range(6)], axis=1)
        y = jnp.dot(z.astype(BF16), gd_v[...], preferred_element_type=F32)
        oa_v[pl.ds(r, RC), :] = y.astype(BF16)
        out_cp(oa_v, 0, r, SEM_OA + i).start()
        return c
    with jax.named_scope("a_rowi"):
        lax.fori_loop(0, NC, a_rowi, 0)

    for i in range(NC):
        out_cp(ob_v, D, i * RC, SEM_OB + i).wait()
    for i in range(NC):
        out_cp(oa_v, 0, i * RC, SEM_OA + i).wait()


@jax.jit
def pallas_concat_heads__spectral_gfnet__sliding_block__prompt_kernel(
    A_x: jax.Array,
    A_w_r: jax.Array,
    A_w_i: jax.Array,
    B_x: jax.Array,
    B_wqkv: jax.Array,
    B_wo: jax.Array,
):
    fd, gd, mf, mi = _tables()
    consts = [jnp.asarray(z, BF16) for z in (fd, gd, mf, mi)]
    any_spec = pl.BlockSpec(memory_space=pl.ANY)
    out = pl.pallas_call(
        _kernel,
        out_shape=jax.ShapeDtypeStruct((S, 2 * D), BF16),
        in_specs=[any_spec] * 10,
        out_specs=any_spec,
        scratch_shapes=[
            pltpu.VMEM((S, D), BF16),
            pltpu.VMEM((DF, S), BF16),
            pltpu.VMEM((DF, S), BF16),
            pltpu.VMEM((S, D), BF16),
            pltpu.VMEM((D, 3 * D), BF16),
            pltpu.VMEM((D, D), BF16),
            pltpu.VMEM((D, 2 * LP), BF16),
            pltpu.VMEM((2 * LP, D), BF16),
            pltpu.VMEM((16, 256, 128), BF16),
            pltpu.VMEM((16, 256, 128), BF16),
            pltpu.VMEM((S, D), BF16),
            pltpu.VMEM((S, D), BF16),
            pltpu.VMEM((S, LP), F32),
            pltpu.VMEM((S, LP), F32),
            pltpu.VMEM((6, S, 128), F32),
            pltpu.VMEM((16, 128, 2 * LP), F32),
            pltpu.VMEM((S, D), BF16),
            pltpu.VMEM((D, S), BF16),
            pltpu.VMEM((D, S), BF16),
            pltpu.VMEM((D, S), F32),
            pltpu.VMEM((2, D, D), BF16),
            pltpu.VMEM((2, H, 3 * BQ, BQ), F32),
            pltpu.SemaphoreType.DMA((24,)),
        ],
        compiler_params=pltpu.CompilerParams(vmem_limit_bytes=110 * 1024 * 1024),
    )(A_x.reshape(S, D), A_w_r.T, A_w_i.T, B_x.reshape(S, D), B_wqkv, B_wo, *consts)
    return out.reshape(1, S, 2 * D)
```

```python
import math

import numpy as np
import jax
import jax.numpy as jnp
from jax import lax
import jax.experimental.pallas as pl
import jax.experimental.pallas.tpu as pltpu

S = 2048
D = 640
DF = 321
LP = 384
H = 32
DH = 20
BQ = 128
F32 = jnp.float32
BF16 = jnp.bfloat16

C1 = math.cos(2.0 * math.pi / 5.0)
C2 = math.cos(4.0 * math.pi / 5.0)
S1 = math.sin(2.0 * math.pi / 5.0)
S2 = math.sin(4.0 * math.pi / 5.0)


def _tables():
    d2 = np.arange(128)[:, None].astype(np.float64)
    l64 = np.arange(64)

    def freqs(k1):
        return np.concatenate([k1 + 5 * l64, (5 - k1) + 5 * l64]).astype(np.float64)

    f0 = np.zeros((128, 256))
    k0 = 5.0 * np.arange(65)[None, :]
    th = 2.0 * np.pi * d2 * k0 / D
    f0[:, 0:65] = np.cos(th)
    f0[:, 128:193] = -np.sin(th)
    fr = [f0]
    for k1 in (1, 2):
        k = freqs(k1)[None, :]
        th = 2.0 * np.pi * d2 * k / D
        co, si = np.cos(th), np.sin(th)
        sg = np.where(np.arange(128) < 64, 1.0, -1.0)[None, :]
        m = np.zeros((256, 256))
        m[:128, :128] = co
        m[128:, :128] = sg * si
        m[:128, 128:] = -si
        m[128:, 128:] = sg * co
        fr.append(m)

    nrm = 1.0 / (S * D)
    g0 = np.zeros((256, 128))
    kk = (5.0 * np.arange(65))[:, None]
    ph = 2.0 * np.pi * kk * d2.T / D
    cc = np.full((65, 1), 2.0)
    cc[0] = 1.0
    cc[64] = 1.0
    g0[0:65, :] = cc * np.cos(ph) * nrm
    gi = -cc * np.sin(ph) * nrm
    gi[0] = 0.0
    gi[64] = 0.0
    g0[128:193, :] = gi
    gr = [g0]
    for k1 in (1, 2):
        k = freqs(k1)[:, None]
        ph = 2.0 * np.pi * k * d2.T / D
        co, si = np.cos(ph), np.sin(ph)
        sg = np.where(np.arange(128) < 64, 1.0, -1.0)[:, None]
        m = np.zeros((256, 256))
        m[:128, :128] = co
        m[128:, :128] = -si
        m[:128, 128:] = sg * si
        m[128:, 128:] = sg * co
        gr.append(2.0 * nrm * m)

    b = np.arange(16)[:, None, None].astype(np.float64)
    k2 = np.arange(128)[None, :, None].astype(np.float64)
    a = np.arange(128)[None, None, :].astype(np.float64)
    th = 2.0 * np.pi * (16.0 * a + b) * k2 / S
    mf = np.concatenate([np.cos(th), -np.sin(th)], axis=1)
    tht = np.transpose(th, (0, 2, 1))
    mi = np.concatenate([np.cos(tht), np.sin(tht)], axis=1)

    f12 = np.stack(fr[1:])
    g12 = np.stack(gr[1:])
    to = lambda z: np.asarray(z, np.float32)
    return [to(z) for z in (fr[0], f12, gr[0], g12, mf, mi)]


def _cmul_const(xr, xi, k, n, sign):
    k = k % n
    if k == 0:
        return xr, xi
    if 4 * k == n:
        return (-xi, xr) if sign > 0 else (xi, -xr)
    if 2 * k == n:
        return -xr, -xi
    if 4 * k == 3 * n:
        return (xi, -xr) if sign > 0 else (-xi, xr)
    cr = math.cos(2.0 * math.pi * k / n)
    ci = sign * math.sin(2.0 * math.pi * k / n)
    if abs(abs(cr) - abs(ci)) < 1e-12:
        if (cr > 0) == (ci > 0):
            return cr * (xr - xi), cr * (xr + xi)
        return cr * (xr + xi), cr * (xi - xr)
    return cr * xr - ci * xi, cr * xi + ci * xr


def _fft_list(xs, sign):
    n = len(xs)
    if n == 1:
        return xs
    ev = _fft_list(xs[0::2], sign)
    od = _fft_list(xs[1::2], sign)
    out = [None] * n
    for k in range(n // 2):
        er, ei = ev[k]
        tr, ti = _cmul_const(od[k][0], od[k][1], k, n, sign)
        out[k] = (er + tr, ei + ti)
        out[k + n // 2] = (er - tr, ei - ti)
    return out


def _kernel(ax_h, wr_h, wi_h, bx_h, wqkv_h, wo_h, f0_h, f12_h, g0_h, g12_h, mf_h, mi_h,
            out_h,
            ax_v, wr_v, wi_v, bx_v, wqkv_v, wo_v, f0_v, f12_v, g0_v, g12_v, mf_v, mi_v,
            oa_v, ob_v, wst, wrn, win,
            u_scr, b_scr, k_scr, k2_scr, qt_scr, vt_scr, ot_scr, wt_scr, s_scr,
            sems):
    RC = 512
    NC = S // RC

    def full_cp(src, dst, i):
        return pltpu.make_async_copy(src, dst, sems.at[i])

    def rows_cp(src, dst, r, i):
        return pltpu.make_async_copy(src.at[pl.ds(r, RC)], dst.at[pl.ds(r, RC)], sems.at[i])

    def out_cp(src, col, r, i):
        return pltpu.make_async_copy(src.at[pl.ds(r, RC)],
                                     out_h.at[pl.ds(r, RC), pl.ds(col, D)], sems.at[i])

    SEM_WQKV, SEM_BX, SEM_WO, SEM_F0, SEM_AX, SEM_WR, SEM_WI = 0, 1, 5, 6, 7, 11, 12
    SEM_MF, SEM_MI, SEM_G0, SEM_OB, SEM_OA, SEM_F12, SEM_G12 = 13, 14, 15, 16, 20, 24, 25

    def slab_cp(j, i):
        return pltpu.make_async_copy(wqkv_h.at[:, pl.ds(j * D, D)],
                                     wqkv_v.at[:, pl.ds(j * D, D)], sems.at[i])

    SEM_WQ, SEM_WV = 26, 27
    slab_cp(1, SEM_WQKV).start()
    rows_cp(bx_h, bx_v, 0, SEM_BX).start()
    for i in range(1, NC):
        rows_cp(bx_h, bx_v, i * RC, SEM_BX + i).start()
    slab_cp(0, SEM_WQ).start()
    slab_cp(2, SEM_WV).start()
    full_cp(f0_h, f0_v, SEM_F0).start()
    full_cp(f12_h, f12_v, SEM_F12).start()
    for i in range(NC):
        rows_cp(ax_h, ax_v, i * RC, SEM_AX + i).start()
    full_cp(wr_h, wr_v, SEM_WR).start()
    full_cp(wi_h, wi_v, SEM_WI).start()
    full_cp(mf_h, mf_v, SEM_MF).start()
    full_cp(wo_h, wo_v, SEM_WO).start()
    full_cp(mi_h, mi_v, SEM_MI).start()
    full_cp(g0_h, g0_v, SEM_G0).start()
    full_cp(g12_h, g12_v, SEM_G12).start()

    slab_cp(1, SEM_WQKV).wait()

    for i in range(NC):
        r = i * RC
        rows_cp(bx_h, bx_v, r, SEM_BX + i).wait()
        if i == 2:
            slab_cp(0, SEM_WQ).wait()
            wt_scr[0] = wqkv_v[:, 0:D].astype(F32).T.astype(BF16)
        if i == 3:
            slab_cp(2, SEM_WV).wait()
            wt_scr[1] = wqkv_v[:, 2 * D:3 * D].astype(F32).T.astype(BF16)
        x = bx_v[pl.ds(r, RC), :]
        kf = jnp.dot(x, wqkv_v[:, D:2 * D], preferred_element_type=F32)
        k_scr[pl.ds(r, RC), :] = kf.astype(BF16)
        k2_scr[pl.ds(r, RC), :] = kf[:, 64:64 + 512].astype(BF16)

    scale = DH ** -0.5
    nt = (((1,), (1,)), ((), ()))

    def b_projqv(i, c):
        r = pl.multiple_of(i * RC, RC)
        x = bx_v[pl.ds(r, RC), :]
        qt = lax.dot_general(wt_scr[0], x, nt, preferred_element_type=F32)
        qt_scr[:, pl.ds(r, RC)] = (qt * scale).astype(BF16)
        vt = lax.dot_general(wt_scr[1], x, nt, preferred_element_type=F32)
        vt_scr[:, pl.ds(r, RC)] = vt.astype(BF16)
        return c
    with jax.named_scope("b_projqv"):
        lax.fori_loop(0, NC, b_projqv, 0)

    full_cp(f0_h, f0_v, SEM_F0).wait()
    full_cp(f12_h, f12_v, SEM_F12).wait()

    def a_row(i, c):
        r = pl.multiple_of(i * RC, RC)
        rows_cp(ax_h, ax_v, r, SEM_AX + i).wait()
        xs = [ax_v[pl.ds(r, RC), j * 128:(j + 1) * 128].astype(F32) for j in range(5)]
        a1 = xs[1] + xs[4]
        a2 = xs[2] + xs[3]
        b1 = xs[1] - xs[4]
        b2 = xs[2] - xs[3]
        t0 = xs[0] + a1 + a2
        t1r = xs[0] + C1 * a1 + C2 * a2
        t1i = -(S1 * b1 + S2 * b2)
        t2r = xs[0] + C2 * a1 + C1 * a2
        t2i = S1 * b2 - S2 * b1
        u0 = jnp.dot(t0.astype(BF16), f0_v[...], preferred_element_type=F32)
        u1 = jnp.dot(jnp.concatenate([t1r, t1i], axis=1).astype(BF16), f12_v[0],
                     preferred_element_type=F32)
        u2 = jnp.dot(jnp.concatenate([t2r, t2i], axis=1).astype(BF16), f12_v[1],
                     preferred_element_type=F32)
        for j, u in enumerate((u0, u1, u2)):
            u_scr[j, pl.ds(r, RC), :] = u[:, :128]
            u_scr[3 + j, pl.ds(r, RC), :] = u[:, 128:]
        return c
    with jax.named_scope("a_row"):
        lax.fori_loop(0, NC, a_row, 0)

    full_cp(wr_h, wr_v, SEM_WR).wait()
    full_cp(wi_h, wi_v, SEM_WI).wait()
    full_cp(mf_h, mf_v, SEM_MF).wait()

    def a_colf(b, c):
        ub = jnp.concatenate([u_scr[j, pl.ds(b, 128, stride=16), :] for j in range(6)],
                             axis=1).astype(BF16)
        pq = jnp.dot(mf_v[b], ub, preferred_element_type=F32)
        p = pq[:128]
        q = pq[128:]
        b_scr[b, :, :LP] = p[:, :LP] - q[:, LP:]
        b_scr[b, :, LP:] = p[:, LP:] + q[:, :LP]
        lanes = pl.ds(pl.multiple_of(b * 128, 128), 128)
        for idx, (src, dst) in enumerate(((wr_v, wrn), (wi_v, win))):
            wst[idx, 0:DF, :] = src[:, lanes].astype(F32)
            blk0 = jnp.concatenate([wst[idx, pl.ds(0, 65, stride=5), :],
                                    jnp.zeros((63, 128), F32)], axis=0)
            blk1 = jnp.concatenate([wst[idx, pl.ds(1, 64, stride=5), :],
                                    wst[idx, pl.ds(4, 64, stride=5), :]], axis=0)
            blk2 = jnp.concatenate([wst[idx, pl.ds(2, 64, stride=5), :],
                                    wst[idx, pl.ds(3, 64, stride=5), :]], axis=0)
            dst[lanes, 0:128] = blk0.T
            dst[lanes, 128:256] = blk1.T
            dst[lanes, 256:384] = blk2.T
        return c
    with jax.named_scope("a_colf"):
        lax.fori_loop(0, 16, a_colf, 0, unroll=16)

    def a_mid(t):
        r = pl.multiple_of(t * 8, 8)
        for lc in range(3):
            lo = lc * 128
            xs = [(b_scr[b, pl.ds(r, 8), lo:lo + 128],
                   b_scr[b, pl.ds(r, 8), LP + lo:LP + lo + 128]) for b in range(16)]
            X = _fft_list(xs, -1)
            Y = []
            for k1 in range(16):
                wr = wrn[pl.ds(128 * k1 + r, 8), lo:lo + 128]
                wi = win[pl.ds(128 * k1 + r, 8), lo:lo + 128]
                xr, xi = X[k1]
                Y.append((xr * wr - xi * wi, xr * wi + xi * wr))
            C = _fft_list(Y, +1)
            for b in range(16):
                b_scr[b, pl.ds(r, 8), lo:lo + 128] = C[b][0]
                b_scr[b, pl.ds(r, 8), LP + lo:LP + lo + 128] = C[b][1]

    jj = lax.broadcasted_iota(jnp.int32, (BQ, BQ), 0)
    ii = lax.broadcasted_iota(jnp.int32, (BQ, BQ), 1)
    tri = jj <= ii

    GROUPS = []
    for h in range(H):
        lo = h * DH
        c0 = (lo // 128) * 128
        key = (0, c0) if lo + DH <= c0 + 128 else (1, c0)
        if GROUPS and GROUPS[-1][0] == key:
            GROUPS[-1][1].append(h)
        else:
            GROUPS.append((key, [h]))

    def qk_group(t, nkb, slot, g):
        ks = t - (nkb - 1) * BQ
        nk = nkb * BQ
        (shifted, c0), heads = GROUPS[g]
        if shifted:
            kk = k2_scr[pl.ds(ks, nk), c0:c0 + 128]
            c0 = c0 + 64
        else:
            kk = k_scr[pl.ds(ks, nk), c0:c0 + 128]
        lanes = lax.broadcasted_iota(jnp.int32, (nk, 128), 1) + c0
        zero = jnp.zeros_like(kk)
        km = jnp.concatenate(
            [jnp.where((lanes >= h * DH) & (lanes < h * DH + DH), kk, zero) for h in heads],
            axis=0)
        qt = qt_scr[c0:c0 + 128, pl.ds(t, BQ)]
        st = jnp.dot(km, qt, preferred_element_type=F32)
        for n, h in enumerate(heads):
            s_scr[slot, h, 0:nk, :] = st[n * nk:(n + 1) * nk]

    def qk_block(t, nkb, slot):
        for g in range(len(GROUPS)):
            qk_group(t, nkb, slot, g)

    def sm_block(t, nkb, slot, heads=range(H)):
        ks = t - (nkb - 1) * BQ
        for h in heads:
            lo = h * DH
            s_last = s_scr[slot, h, (nkb - 1) * BQ:nkb * BQ, :]
            if nkb == 3:
                cmb = jnp.where(tri, s_last, s_scr[slot, h, 0:BQ, :])
            else:
                cmb = jnp.where(tri, s_last, -1e30)
            m = jnp.max(cmb, axis=0, keepdims=True)
            if nkb >= 2:
                s_mid = s_scr[slot, h, (nkb - 2) * BQ:(nkb - 1) * BQ, :]
                m = jnp.maximum(m, jnp.max(s_mid, axis=0, keepdims=True))
            pc = jnp.exp(cmb - m)
            l = jnp.sum(pc, axis=0, keepdims=True)
            p_last = jnp.where(tri, pc, 0.0).astype(BF16)
            vt = vt_scr[lo:lo + DH, pl.ds(ks, nkb * BQ)]
            o = jnp.dot(vt[:, (nkb - 1) * BQ:], p_last, preferred_element_type=F32)
            if nkb >= 2:
                pm = jnp.exp(s_mid - m)
                l = l + jnp.sum(pm, axis=0, keepdims=True)
                o = o + jnp.dot(vt[:, (nkb - 2) * BQ:(nkb - 1) * BQ], pm.astype(BF16),
                                preferred_element_type=F32)
            if nkb == 3:
                p_first = jnp.where(tri, 0.0, pc).astype(BF16)
                o = o + jnp.dot(vt[:, :BQ], p_first, preferred_element_type=F32)
            ot_scr[lo:lo + DH, pl.ds(t, BQ)] = o / l

    qk_block(0, 1, 0)
    for g in range(len(GROUPS)):
        qk_group(BQ, 2, 1, g)
        sm_block(0, 1, 0, GROUPS[g][1])
    for g in range(len(GROUPS)):
        qk_group(2 * BQ, 3, 0, g)
        sm_block(BQ, 2, 1, GROUPS[g][1])

    def attn_loop(j, c):
        t = pl.multiple_of((2 * j + 3) * BQ, BQ)
        for g in range(len(GROUPS)):
            qk_group(t, 3, 1, g)
            sm_block(t - BQ, 3, 0, GROUPS[g][1])
        for g in range(len(GROUPS)):
            qk_group(t + BQ, 3, 0, g)
            sm_block(t, 3, 1, GROUPS[g][1])
        return c
    with jax.named_scope("attn_loop"):
        lax.fori_loop(0, 6, attn_loop, 0)
    for g in range(len(GROUPS)):
        qk_group(15 * BQ, 3, 1, g)
        sm_block(14 * BQ, 3, 0, GROUPS[g][1])
    sm_block(15 * BQ, 3, 1)

    full_cp(wo_h, wo_v, SEM_WO).wait()

    def b_out(i, c):
        r = pl.multiple_of(i * RC, RC)
        o = ot_scr[:, pl.ds(r, RC)].T.astype(BF16)
        y = jnp.dot(o, wo_v[...], preferred_element_type=F32)
        ob_v[pl.ds(r, RC), :] = y.astype(BF16)
        out_cp(ob_v, D, r, SEM_OB + i).start()
        for tt in range(4):
            a_mid(i * 4 + tt)
        return c
    with jax.named_scope("b_out"):
        lax.fori_loop(0, NC, b_out, 0)

    full_cp(mi_h, mi_v, SEM_MI).wait()

    def a_coli(b, c):
        cb = b_scr[b].astype(BF16)
        pq = jnp.dot(mi_v[b], cb, preferred_element_type=F32)
        p = pq[:128]
        q = pq[128:]
        zr = p[:, :LP] - q[:, LP:]
        zi = p[:, LP:] + q[:, :LP]
        for j in range(3):
            u_scr[j, pl.ds(b, 128, stride=16), :] = zr[:, j * 128:(j + 1) * 128]
            u_scr[3 + j, pl.ds(b, 128, stride=16), :] = zi[:, j * 128:(j + 1) * 128]
        return c
    with jax.named_scope("a_coli"):
        lax.fori_loop(0, 16, a_coli, 0, unroll=16)

    full_cp(g0_h, g0_v, SEM_G0).wait()
    full_cp(g12_h, g12_v, SEM_G12).wait()

    def a_rowi(i, c):
        r = pl.multiple_of(i * RC, RC)
        zs = [jnp.concatenate([u_scr[j, pl.ds(r, RC), :], u_scr[3 + j, pl.ds(r, RC), :]],
                              axis=1).astype(BF16) for j in range(3)]
        g0 = jnp.dot(zs[0], g0_v[...], preferred_element_type=F32)
        g1 = jnp.dot(zs[1], g12_v[0], preferred_element_type=F32)
        g2 = jnp.dot(zs[2], g12_v[1], preferred_element_type=F32)
        g1r, g1i = g1[:, :128], g1[:, 128:]
        g2r, g2i = g2[:, :128], g2[:, 128:]
        e1 = g0 + C1 * g1r + C2 * g2r
        f1 = S1 * g1i + S2 * g2i
        e2 = g0 + C2 * g1r + C1 * g2r
        f2 = S2 * g1i - S1 * g2i
        ys = (g0 + g1r + g2r, e1 - f1, e2 - f2, e2 + f2, e1 + f1)
        for j in range(5):
            oa_v[pl.ds(r, RC), j * 128:(j + 1) * 128] = ys[j].astype(BF16)
        out_cp(oa_v, 0, r, SEM_OA + i).start()
        return c
    with jax.named_scope("a_rowi"):
        lax.fori_loop(0, NC, a_rowi, 0)

    for i in range(NC):
        out_cp(ob_v, D, i * RC, SEM_OB + i).wait()
    for i in range(NC):
        out_cp(oa_v, 0, i * RC, SEM_OA + i).wait()


@jax.jit
def pallas_concat_heads__spectral_gfnet__sliding_block__prompt_kernel(
    A_x: jax.Array,
    A_w_r: jax.Array,
    A_w_i: jax.Array,
    B_x: jax.Array,
    B_wqkv: jax.Array,
    B_wo: jax.Array,
):
    consts = [jnp.asarray(z, BF16) for z in _tables()]
    any_spec = pl.BlockSpec(memory_space=pl.ANY)
    out = pl.pallas_call(
        _kernel,
        out_shape=jax.ShapeDtypeStruct((S, 2 * D), BF16),
        in_specs=[any_spec] * 12,
        out_specs=any_spec,
        scratch_shapes=[
            pltpu.VMEM((S, D), BF16),
            pltpu.VMEM((DF, S), BF16),
            pltpu.VMEM((DF, S), BF16),
            pltpu.VMEM((S, D), BF16),
            pltpu.VMEM((D, 3 * D), BF16),
            pltpu.VMEM((D, D), BF16),
            pltpu.VMEM((128, 256), BF16),
            pltpu.VMEM((2, 256, 256), BF16),
            pltpu.VMEM((256, 128), BF16),
            pltpu.VMEM((2, 256, 256), BF16),
            pltpu.VMEM((16, 256, 128), BF16),
            pltpu.VMEM((16, 256, 128), BF16),
            pltpu.VMEM((S, D), BF16),
            pltpu.VMEM((S, D), BF16),
            pltpu.VMEM((2, 328, 128), F32),
            pltpu.VMEM((S, LP), F32),
            pltpu.VMEM((S, LP), F32),
            pltpu.VMEM((6, S, 128), F32),
            pltpu.VMEM((16, 128, 2 * LP), F32),
            pltpu.VMEM((S, D), BF16),
            pltpu.VMEM((S, 512), BF16),
            pltpu.VMEM((D, S), BF16),
            pltpu.VMEM((D, S), BF16),
            pltpu.VMEM((D, S), F32),
            pltpu.VMEM((2, D, D), BF16),
            pltpu.VMEM((2, H, 3 * BQ, BQ), F32),
            pltpu.SemaphoreType.DMA((28,)),
        ],
        compiler_params=pltpu.CompilerParams(vmem_limit_bytes=110 * 1024 * 1024),
    )(A_x.reshape(S, D), A_w_r.T, A_w_i.T, B_x.reshape(S, D), B_wqkv, B_wo, *consts)
    return out.reshape(1, S, 2 * D)
```
